```python
import jax
import jax.numpy as jnp

def _softmax(x, axis=-1):
    return jax.nn.softmax(x, axis=axis)
def _gelu(x):
    return jax.nn.gelu(x, approximate=True)
def _silu(x):
    return jax.nn.silu(x)
def _sigmoid(x):
    return jax.nn.sigmoid(x)
def _layernorm(x, axis=-1, eps=1e-5):
    m = jnp.mean(x, axis=axis, keepdims=True)
    v = jnp.var(x, axis=axis, keepdims=True)
    return (x - m) / jnp.sqrt(v + eps)
def _scatter_add(tgt, idx, src, axis=0):
    return tgt.at[idx].add(src)
def _segment_sum(src, seg, n):
    return jax.ops.segment_sum(src, seg, n)
class _Rng:
    def __init__(self, key):
        self._k = key
    def _next(self):
        self._k, sub = jax.random.split(self._k)
        return sub
    def normal(self, shape):
        return jax.random.normal(self._next(), shape, dtype=jnp.bfloat16)
    def randint(self, lo, hi, shape):
        return jax.random.randint(self._next(), shape, lo, hi, dtype=jnp.int32)
    def uniform(self, shape, lo=0.0, hi=1.0):
        return jax.random.uniform(self._next(), shape, jnp.bfloat16, lo, hi)
    def permutation(self, n):
        return jax.random.permutation(self._next(), n)


kernel_name = 'gated_mix__sliding_block_cached__moe_arch_mod__decode'

def setup_inputs():
    _rng = _Rng(jax.random.key(int.from_bytes(__import__("os").urandom(4), "little")))
    _w = (lambda a: (lambda t: t.astype(jnp.bfloat16) if jnp.issubdtype(t.dtype, jnp.floating) else t)(jnp.asarray(a)))
    def _A_setup():
        B, Sq, D = 1, 1, 640
        Hq, Hkv, Sk, Dh = 32, 32, 32768, 192
        assert Hq % Hkv == 0, (Hq, Hkv)
        return {
            "x": _w((lambda *s: _rng.normal(s) * 0.05)(B, Sq, D)),
            "k_cache": _w((lambda *s: _rng.normal(s) * 0.05)(B, Hkv, Sk, Dh)),
            "v_cache": _w((lambda *s: _rng.normal(s) * 0.05)(B, Hkv, Sk, Dh)),
            "wq": _w((lambda *s: _rng.normal(s) * 0.05)(D, Hq * Dh) * (D ** -0.5)),
            "wo": _w((lambda *s: _rng.normal(s) * 0.05)(Hq * Dh, D) * ((Hq * Dh) ** -0.5)),
        }
    _A_in = _A_setup()

    def _B_setup():
        B, S, D, F, C = 1, 1, 640, 1536, 1
        return {
            "x": _w((lambda *s: _rng.normal(s) * 0.05)(B, S, D)),
            "w_r": _w((lambda *s: _rng.normal(s) * 0.05)(D)),
            "w_gate": _w((lambda *s: _rng.normal(s) * 0.05)(D, F)),
            "w_up": _w((lambda *s: _rng.normal(s) * 0.05)(D, F)),
            "w_down": _w((lambda *s: _rng.normal(s) * 0.05)(F, D)),
        }
    _B_in = _B_setup()

    return {
        "A_x": _A_in["x"],
        "A_k_cache": _A_in["k_cache"],
        "A_v_cache": _A_in["v_cache"],
        "A_wq": _A_in["wq"],
        "A_wo": _A_in["wo"],
        "B_x": _B_in["x"],
        "B_w_r": _B_in["w_r"],
        "B_w_gate": _B_in["w_gate"],
        "B_w_up": _B_in["w_up"],
        "B_w_down": _B_in["w_down"],
        "gate_w": _w((lambda *s: _rng.normal(s) * 0.05)(640)),
    }

def reference(A_x, A_k_cache, A_v_cache, A_wq, A_wo, B_x, B_w_r, B_w_gate, B_w_up, B_w_down, gate_w):
    def _A_ref(x, k_cache, v_cache, wq, wo):
        B, Sq, D = x.shape
        Hq, Dh = 32, 192
        Hkv, Sk = k_cache.shape[1], k_cache.shape[2]
        W = min(4096, max(256, Sk // 4))
        rep = Hq // Hkv
        q = (lambda x, *d: x.transpose(*d))((x @ wq).reshape(B, Sq, Hq, Dh), 0, 2, 1, 3)
        k = jnp.repeat(k_cache[:, :, Sk - W:, :], rep, axis=1)
        v = jnp.repeat(v_cache[:, :, Sk - W:, :], rep, axis=1)
        scores = jnp.einsum("bhqd,bhkd->bhqk", q, k) * (Dh ** -0.5)
        p = _softmax(scores, axis=-1)
        o = jnp.einsum("bhqk,bhkd->bhqd", p, v)
        return (lambda x, *d: x.transpose(*d))(o, 0, 2, 1, 3).reshape(B, Sq, Hq * Dh) @ wo

    def _B_ref(x, w_r, w_gate, w_up, w_down):
        B, S, D = x.shape
        C = 1
        r = x @ w_r
        idx = jnp.argsort(-r, axis=-1)[:, :C]
        idx_e = jnp.repeat(idx.reshape(B, C, 1), D, axis=2)
        x_sel = jnp.take_along_axis(x, idx_e, axis=1)
        g = _silu(x_sel @ w_gate)
        u = x_sel @ w_up
        y = (g * u) @ w_down
        r_sel = _sigmoid(jnp.take_along_axis(r, idx, axis=1))
        y = y * r_sel.reshape(B, C, 1)
        b_off = (jnp.arange(B) * S).reshape(B, 1)
        flat_idx = (idx + b_off).reshape(B * C)
        zero = (x * 0.0).reshape(B * S, D)
        upd = _scatter_add(zero, flat_idx, y.reshape(B * C, D), axis=0)
        return x + upd.reshape(B, S, D)

    x = A_x
    g = _sigmoid((x * gate_w).sum(-1, keepdims=True))
    a = _A_ref(x, A_k_cache, A_v_cache, A_wq, A_wo)
    b = _B_ref(x, B_w_r, B_w_gate, B_w_up, B_w_down)
    return g * a + (1 - g) * b
```

```python
import functools
import jax
import jax.numpy as jnp
import numpy as np
import jax.experimental.pallas as pl
import jax.experimental.pallas.tpu as pltpu

HQ, DH = 32, 192
F32, BF16 = jnp.float32, jnp.bfloat16


def _rb(v):
    return v.astype(BF16).astype(F32)


def _pieces(R, C, pr, pc, order):
    rs = range(0, R, pr)
    cs = range(0, C, pc)
    if order == 'rl':
        return [(r, c) for r in rs for c in cs]
    return [(r, c) for c in cs for r in rs]


def _kernel(x_hbm, k_hbm, v_hbm, wq_hbm, wo_hbm, wr_hbm, wg_hbm, wu_hbm, wd_hbm, gw_hbm,
            o_ref,
            x_v, wr_v, gw_v, wq_v, wo_v, wg_v, wu_v, wd_v, kbuf, vbuf, q_v,
            wsem, dsem, ksem, vsem, *, nbuf, s0, w, kvp, nwd, pre):
    H = HQ
    D = x_hbm.shape[-1]
    Fd = wg_hbm.shape[1]
    pr, pc, order = kvp

    def start_kv(src, dst, sem, h, slot):
        for n, (r, c) in enumerate(_pieces(DH, w, pr, pc, order)):
            pltpu.make_async_copy(
                src.at[0, h, pl.ds(r, pr), pl.ds(s0 + c, pc)],
                dst.at[slot, pl.ds(r, pr), pl.ds(c, pc)],
                sem.at[slot]).start(priority=n % 2)

    def wait_all(dst, sem):
        pltpu.make_async_copy(dst, dst, sem).wait()

    def start_halves(src, dst, sem, row0, nrows, rows, cols):
        half = nrows // 2
        ncol = src.shape[1] // cols

        @pl.loop(0, half // rows)
        def _(i):
            for c in range(ncol):
                for t in range(2):
                    r = pl.multiple_of(row0 + t * half + i * rows, 8)
                    pltpu.make_async_copy(
                        src.at[pl.ds(r, rows), pl.ds(c * cols, cols)],
                        dst.at[pl.ds(r, rows), pl.ds(c * cols, cols)], sem).start(priority=t)

    def start_pair(srcs, dsts, sem, rows):
        @pl.loop(0, srcs[0].shape[0] // rows)
        def _(i):
            r = pl.multiple_of(i * rows, 8)
            for t in range(2):
                pltpu.make_async_copy(srcs[t].at[pl.ds(r, rows), :], dsts[t].at[pl.ds(r, rows), :], sem).start(priority=t)

    c_x = pltpu.make_async_copy(x_hbm, x_v, wsem.at[0])
    c_wr = pltpu.make_async_copy(wr_hbm, wr_v, wsem.at[0])
    c_gw = pltpu.make_async_copy(gw_hbm, gw_v, wsem.at[0])
    c_x.start(); c_wr.start(); c_gw.start()
    start_halves(wq_hbm, wq_v, wsem.at[0], 0, D, 8, 2048)
    start_pair((wg_hbm, wu_hbm), (wg_v, wu_v), wsem.at[1], 8)

    @pl.loop(0, pre)
    def _(u):
        h = u // 2
        @pl.when(u % 2 == 0)
        def _():
            start_kv(k_hbm, kbuf, ksem, h, h)
        @pl.when(u % 2 == 1)
        def _():
            start_kv(v_hbm, vbuf, vsem, h, h)

    c_x.wait(); c_wr.wait(); c_gw.wait()
    wait_all(wq_v, wsem.at[0])
    x1 = x_v[0]
    x8 = jnp.broadcast_to(x1, (8, D))
    q = jnp.dot(x8, wq_v[...], preferred_element_type=F32)
    q = _rb(q)
    for h in range(H):
        q_v[h] = q[:, h * DH:(h + 1) * DH]

    @pl.loop(pre, 2 * nbuf)
    def _(u):
        h = u // 2
        @pl.when(u % 2 == 0)
        def _():
            start_kv(k_hbm, kbuf, ksem, h, h)
        @pl.when(u % 2 == 1)
        def _():
            start_kv(v_hbm, vbuf, vsem, h, h)

    xf = x1.astype(F32)
    wr = wr_v[...].reshape(1, D).astype(F32)
    gw = gw_v[...].reshape(1, D).astype(F32)
    r = _rb(jnp.sum(xf * wr, axis=-1, keepdims=True))
    r_sel = _rb(jax.nn.sigmoid(r))
    gsum = _rb(jnp.sum(_rb(xf * gw), axis=-1, keepdims=True))
    g = _rb(jax.nn.sigmoid(gsum))
    wait_all(wg_v, wsem.at[1])
    wait_all(wu_v, wsem.at[1])
    gate = _rb(jnp.dot(x8, wg_v[...], preferred_element_type=F32))
    up = _rb(jnp.dot(x8, wu_v[...], preferred_element_type=F32))
    hmid = (_rb(jax.nn.silu(gate)) * up).astype(BF16)

    start_halves(wo_hbm, wo_v, wsem.at[2], 0, H * DH, 24, D)
    wait_all(wo_v, wsem.at[2])

    scale = np.float32(np.asarray(DH ** -0.5, dtype=jnp.bfloat16))
    wd_rows = Fd // nwd

    def head(h, acc):
        slot = h % nbuf
        wait_all(kbuf.at[slot], ksem.at[slot])
        qh = q_v[h].astype(BF16)
        s = jnp.dot(qh, kbuf[slot], preferred_element_type=F32) * scale

        @pl.when(h + nbuf < H)
        def _():
            start_kv(k_hbm, kbuf, ksem, h + nbuf, slot)

        m = jnp.max(s, axis=-1, keepdims=True)
        p = jnp.exp(s - m)
        l = jnp.sum(p, axis=-1, keepdims=True)
        wait_all(vbuf.at[slot], vsem.at[slot])
        pv = jax.lax.dot_general(p.astype(BF16), vbuf[slot], (((1,), (1,)), ((), ())),
                                 preferred_element_type=F32)

        @pl.when(h + nbuf < H)
        def _():
            start_kv(v_hbm, vbuf, vsem, h + nbuf, slot)

        @pl.when(h + nbuf == H)
        def _():
            for j in range(nwd):
                start_halves(wd_hbm, wd_v, dsem.at[j], j * wd_rows, wd_rows, 32, D)

        o = (pv / l).astype(BF16)
        row0 = pl.multiple_of(h * DH, 64)
        return acc + jnp.dot(o, wo_v[pl.ds(row0, DH), :], preferred_element_type=F32)

    acc = jax.lax.fori_loop(0, H, head, jnp.zeros((8, D), F32))
    a = _rb(acc[0:1])
    ga = _rb(g * a)
    omg = _rb(1.0 - g)
    y = jnp.zeros((8, D), F32)
    for j in range(nwd):
        rows = pl.ds(j * wd_rows, wd_rows)
        wait_all(wd_v.at[rows, :], dsem.at[j])
        y = y + jnp.dot(hmid[:, j * wd_rows:(j + 1) * wd_rows], wd_v[rows, :], preferred_element_type=F32)
    y = _rb(_rb(y[0:1]) * r_sel)
    b = _rb(xf + _rb(_rb(xf * 0.0) + y))
    out = ga + _rb(omg * b)
    o_ref[0] = out.astype(o_ref.dtype)


@jax.jit
def pallas_gated_mix__sliding_block_cached__moe_arch_mod__decode_kernel(
    A_x, A_k_cache, A_v_cache, A_wq, A_wo, B_x, B_w_r, B_w_gate, B_w_up, B_w_down, gate_w,
):
    nbuf, kvp, nwd, pre = 2, (24, 512, 'lr'), 3, 2
    del B_x
    Bsz, Sq, D = A_x.shape
    Sk = A_k_cache.shape[2]
    W = min(4096, max(256, Sk // 4))
    F = B_w_gate.shape[1]
    any_spec = pl.BlockSpec(memory_space=pl.ANY)
    return pl.pallas_call(
        functools.partial(_kernel, nbuf=nbuf, s0=Sk - W, w=W, kvp=kvp, nwd=nwd, pre=pre),
        in_specs=[any_spec] * 10,
        out_specs=pl.BlockSpec(memory_space=pltpu.VMEM),
        out_shape=jax.ShapeDtypeStruct((Bsz, Sq, D), A_x.dtype),
        scratch_shapes=[
            pltpu.VMEM((1, 1, D), BF16),
            pltpu.VMEM((D,), BF16),
            pltpu.VMEM((D,), BF16),
            pltpu.VMEM((D, HQ * DH), BF16),
            pltpu.VMEM((HQ * DH, D), BF16),
            pltpu.VMEM((D, F), BF16),
            pltpu.VMEM((D, F), BF16),
            pltpu.VMEM((F, D), BF16),
            pltpu.VMEM((nbuf, DH, W), BF16),
            pltpu.VMEM((nbuf, DH, W), BF16),
            pltpu.VMEM((HQ, 8, DH), F32),
            pltpu.SemaphoreType.DMA((3,)),
            pltpu.SemaphoreType.DMA((nwd,)),
            pltpu.SemaphoreType.DMA((nbuf,)),
            pltpu.SemaphoreType.DMA((nbuf,)),
        ],
        compiler_params=pltpu.CompilerParams(vmem_limit_bytes=100 * 1024 * 1024),
        name="gated_mix_decode",
    )(A_x, A_k_cache.transpose(0, 1, 3, 2), A_v_cache.transpose(0, 1, 3, 2), A_wq, A_wo,
      B_w_r, B_w_gate, B_w_up, B_w_down, gate_w)
```

```python
import functools
import jax
import jax.numpy as jnp
import numpy as np
import jax.experimental.pallas as pl
import jax.experimental.pallas.tpu as pltpu

HQ, DH = 32, 192
F32, BF16 = jnp.float32, jnp.bfloat16


def _rb(v):
    return v.astype(BF16).astype(F32)


def _pieces(R, C, pr, pc, order):
    nr, nl = R // pr, C // pc
    if order == 'rl':
        idx = [(i, j) for i in range(nr) for j in range(nl)]
    elif order == 'lr':
        idx = [(i, j) for j in range(nl) for i in range(nr)]
    else:
        idx = [(i, (j + i) % nl) for j in range(nl) for i in range(nr)]
    return [(i * pr, j * pc) for i, j in idx]


def _kernel(x_hbm, k_hbm, v_hbm, wq_hbm, wo_hbm, wr_hbm, wg_hbm, wu_hbm, wd_hbm, gw_hbm,
            o_ref,
            x_v, wr_v, gw_v, wq_v, wo_v, wg_v, wu_v, wd_v, kbuf, vbuf, q_v, hm_v,
            wsem, dsem, ksem, vsem, *, nbuf, s0, w, kvp, nwd, wd_pr, pre, nocompute, wo_first):
    H = HQ
    D = x_hbm.shape[-1]
    Fd = wg_hbm.shape[1]
    pr, pc, order = kvp

    def start_kv(src, dst, sem, h, slot):
        for n, (r, c) in enumerate(_pieces(DH, w, pr, pc, order)):
            pltpu.make_async_copy(
                src.at[0, h, pl.ds(r, pr), pl.ds(s0 + c, pc)],
                dst.at[slot, pl.ds(r, pr), pl.ds(c, pc)],
                sem.at[slot]).start(priority=n % 2)

    def wait_all(dst, sem):
        pltpu.make_async_copy(dst, dst, sem).wait()

    def copy(src, dst, sem, r, nr, c, nc, prio):
        pltpu.make_async_copy(src.at[pl.ds(r, nr), pl.ds(c, nc)], dst.at[pl.ds(r, nr), pl.ds(c, nc)], sem).start(priority=prio)

    def start_wq():
        nrt = D // 8
        st = 5
        cw = H * DH // 3

        @pl.loop(0, 3)
        def _(cc):
            @pl.loop(0, st)
            def _(j):
                for i in range(nrt // st):
                    r = pl.multiple_of((i * st + j) * 8, 8)
                    c = pl.multiple_of(cc * cw, 128)
                    copy(wq_hbm, wq_v, wsem.at[0], r, 8, c, cw, i % 2)

    def start_wgu():
        npc = D // 8
        st = 20

        @pl.loop(0, st)
        def _(j):
            for i in range(npc // st):
                r = pl.multiple_of((i * st + j) * 8, 8)
                copy(wg_hbm, wg_v, wsem.at[1], r, 8, 0, Fd, 0)
                copy(wu_hbm, wu_v, wsem.at[1], r, 8, 0, Fd, 1)

    def start_wo(j0, j1):
        @pl.loop(j0, j1)
        def _(j):
            for i in range(16):
                r = pl.multiple_of(384 * i + 24 * j, 8)
                copy(wo_hbm, wo_v, wsem.at[2], r, 24, 0, D, i % 2)

    wd_rows = Fd // nwd

    def start_wd():
        rows = wd_pr
        half = wd_rows // rows // 2

        @pl.loop(0, nwd)
        def _(jj):
            for i in range(half):
                for t in range(2):
                    r = pl.multiple_of(jj * wd_rows + (t * half + i) * rows, 8)
                    copy(wd_hbm, wd_v, dsem.at[jj], r, rows, 0, D, t)

    def start_units(lo, hi):
        @pl.loop(lo, hi)
        def _(u):
            h = u >> 1
            @pl.when(u & 1 == 0)
            def _():
                start_kv(k_hbm, kbuf, ksem, h, h)
            @pl.when(u & 1 == 1)
            def _():
                start_kv(v_hbm, vbuf, vsem, h, h)

    c_x = pltpu.make_async_copy(x_hbm, x_v, wsem.at[0])
    c_wr = pltpu.make_async_copy(wr_hbm, wr_v, wsem.at[0])
    c_gw = pltpu.make_async_copy(gw_hbm, gw_v, wsem.at[0])
    start_wq()
    c_x.start(priority=0); c_wr.start(priority=1); c_gw.start(priority=0)
    start_wgu()
    start_units(0, pre)

    c_x.wait(); c_wr.wait(); c_gw.wait()
    wait_all(wq_v, wsem.at[0])
    if not nocompute:
        x1 = x_v[0]
        x8 = jnp.broadcast_to(x1, (8, D))
        q = jnp.dot(x8, wq_v[...], preferred_element_type=F32)
        q = _rb(q)
        for h in range(H):
            q_v[h] = q[:, h * DH:(h + 1) * DH]

    start_wo(0, wo_first)

    wait_all(wg_v, wsem.at[1])
    wait_all(wu_v, wsem.at[1])
    if not nocompute:
        xf = x1.astype(F32)
        wr = wr_v[...].reshape(1, D).astype(F32)
        gw = gw_v[...].reshape(1, D).astype(F32)
        r_sel = jax.nn.sigmoid(jnp.sum(xf * wr, axis=-1, keepdims=True))
        g = jax.nn.sigmoid(jnp.sum(xf * gw, axis=-1, keepdims=True))
        gate = jnp.dot(x8, wg_v[...], preferred_element_type=F32)
        up = jnp.dot(x8, wu_v[...], preferred_element_type=F32)
        hmid = _rb(jax.nn.silu(gate) * up)
        for j in range(nwd):
            hm_v[j] = hmid[:, j * wd_rows:(j + 1) * wd_rows]

    start_wo(wo_first, 16)
    start_units(pre, 2 * nbuf)
    wait_all(wo_v, wsem.at[2])

    scale = np.float32(DH ** -0.5)

    def head(h, acc):
        slot = h % nbuf
        wait_all(kbuf.at[slot], ksem.at[slot])
        if not nocompute:
            qh = q_v[h].astype(BF16)
            s = jnp.dot(qh, kbuf[slot], preferred_element_type=F32) * scale

        @pl.when(h + nbuf < H)
        def _():
            start_kv(k_hbm, kbuf, ksem, h + nbuf, slot)

        if not nocompute:
            m = jnp.max(s, axis=-1, keepdims=True)
            p = jnp.exp(s - m)
            l = jnp.sum(p, axis=-1, keepdims=True)
        wait_all(vbuf.at[slot], vsem.at[slot])
        if not nocompute:
            pv = jax.lax.dot_general(p.astype(BF16), vbuf[slot], (((1,), (1,)), ((), ())),
                                     preferred_element_type=F32)

        @pl.when(h + nbuf < H)
        def _():
            start_kv(v_hbm, vbuf, vsem, h + nbuf, slot)

        @pl.when(h + nbuf == H)
        def _():
            start_wd()

        if nocompute:
            return acc
        o = (pv / l).astype(BF16)
        row0 = pl.multiple_of(h * DH, 64)
        return acc + jnp.dot(o, wo_v[pl.ds(row0, DH), :], preferred_element_type=F32)

    acc = jax.lax.fori_loop(0, H, head, jnp.zeros((8, D), F32))
    def wd_wait(j):
        r = pl.multiple_of(j * wd_rows, wd_rows)
        rows = pl.ds(r, wd_rows)
        wait_all(wd_v.at[rows, :], dsem.at[j])
        return rows

    if nocompute:
        @pl.loop(0, nwd)
        def _(j):
            wd_wait(j)
        o_ref[...] = jnp.zeros(o_ref.shape, o_ref.dtype)
        return
    ga = g * acc[0:1]
    omg = 1.0 - g
    base = xf + xf * 0.0

    def down(j, y):
        rows = wd_wait(j)
        return y + jnp.dot(hm_v[j].astype(BF16), wd_v[rows, :], preferred_element_type=F32)

    y = jax.lax.fori_loop(0, nwd, down, jnp.zeros((8, D), F32))
    b = base + y[0:1] * r_sel
    o_ref[0] = (ga + omg * b).astype(o_ref.dtype)


@jax.jit
def pallas_gated_mix__sliding_block_cached__moe_arch_mod__decode_kernel(
    A_x, A_k_cache, A_v_cache, A_wq, A_wo, B_x, B_w_r, B_w_gate, B_w_up, B_w_down, gate_w,
):
    nbuf, kvp, nwd, wd_pr, pre, dbc, nocompute, wo_first = 2, (8, 2048, 'diag'), 4, 24, 2, False, False, 4
    del B_x
    Bsz, Sq, D = A_x.shape
    Sk = A_k_cache.shape[2]
    W = min(4096, max(256, Sk // 4))
    F = B_w_gate.shape[1]
    any_spec = pl.BlockSpec(memory_space=pl.ANY)
    return pl.pallas_call(
        functools.partial(_kernel, nbuf=nbuf, s0=Sk - W, w=W, kvp=kvp, nwd=nwd, wd_pr=wd_pr, pre=pre, nocompute=nocompute, wo_first=wo_first),
        in_specs=[any_spec] * 10,
        out_specs=pl.BlockSpec(memory_space=pltpu.VMEM),
        out_shape=jax.ShapeDtypeStruct((Bsz, Sq, D), A_x.dtype),
        scratch_shapes=[
            pltpu.VMEM((1, 1, D), BF16),
            pltpu.VMEM((D,), BF16),
            pltpu.VMEM((D,), BF16),
            pltpu.VMEM((D, HQ * DH), BF16),
            pltpu.VMEM((HQ * DH, D), BF16),
            pltpu.VMEM((D, F), BF16),
            pltpu.VMEM((D, F), BF16),
            pltpu.VMEM((F, D), BF16),
            pltpu.VMEM((nbuf, DH, W), BF16),
            pltpu.VMEM((nbuf, DH, W), BF16),
            pltpu.VMEM((HQ, 8, DH), F32),
            pltpu.VMEM((nwd, 8, F // nwd), F32),
            pltpu.SemaphoreType.DMA((3,)),
            pltpu.SemaphoreType.DMA((nwd,)),
            pltpu.SemaphoreType.DMA((nbuf,)),
            pltpu.SemaphoreType.DMA((nbuf,)),
        ],
        compiler_params=pltpu.CompilerParams(vmem_limit_bytes=100 * 1024 * 1024, disable_bounds_checks=dbc),
        name="gated_mix_decode",
    )(A_x, A_k_cache.transpose(0, 1, 3, 2), A_v_cache.transpose(0, 1, 3, 2), A_wq, A_wo,
      B_w_r, B_w_gate, B_w_up, B_w_down, gate_w)
```

```python
import functools

import jax
import jax.numpy as jnp
import numpy as np
import jax.experimental.pallas as pl
import jax.experimental.pallas.tpu as pltpu

HQ, DH = 32, 192
F32, BF16 = jnp.float32, jnp.bfloat16

NBUF = 2
KV_LANES = 2048
N_DOWN = 4


def _rb(v):
    return v.astype(BF16).astype(F32)


def _kernel(x_hbm, k_hbm, v_hbm, wq_hbm, wo_hbm, wr_hbm, wg_hbm, wu_hbm, wd_hbm, gw_hbm,
            o_ref,
            x_v, wr_v, gw_v, wq_v, wo_v, wg_v, wu_v, wd_v, kbuf, vbuf, q_v, hm_v,
            wsem, dsem, ksem, vsem, *, s0, w):
    H = HQ
    D = x_hbm.shape[-1]
    Fd = wg_hbm.shape[1]
    down_rows = Fd // N_DOWN

    def copy(src, dst, sem, r, nr, c, nc, prio):
        pltpu.make_async_copy(src.at[pl.ds(r, nr), pl.ds(c, nc)],
                              dst.at[pl.ds(r, nr), pl.ds(c, nc)], sem).start(priority=prio)

    def wait_all(dst, sem):
        pltpu.make_async_copy(dst, dst, sem).wait()

    def strided(n_pieces, stride, j0, j1, issue):
        inner = n_pieces // stride
        assert inner * stride == n_pieces and inner % 2 == 0

        @pl.loop(j0, j1)
        def _(j):
            for i in range(inner):
                issue(i * stride + j, i % 2)

    def start_kv(src, dst, sem, h, slot):
        n = 0
        for c in range(0, w, KV_LANES):
            for r in range(0, DH, 8):
                pltpu.make_async_copy(
                    src.at[0, h, pl.ds(r, 8), pl.ds(s0 + c, KV_LANES)],
                    dst.at[slot, pl.ds(r, 8), pl.ds(c, KV_LANES)],
                    sem.at[slot]).start(priority=n % 2)
                n += 1

    def start_units(lo, hi):
        @pl.loop(lo, hi)
        def _(u):
            h = u >> 1

            @pl.when((u & 1) == 0)
            def _():
                start_kv(k_hbm, kbuf, ksem, h, h)

            @pl.when((u & 1) == 1)
            def _():
                start_kv(v_hbm, vbuf, vsem, h, h)

    wq_cols = H * DH // 3

    def issue_wq(p, prio):
        rt = (p * 43691) >> 17
        c = p - 3 * rt
        copy(wq_hbm, wq_v, wsem.at[0], pl.multiple_of(rt * 8, 8), 8,
             pl.multiple_of(c * wq_cols, 128), wq_cols, prio)

    def issue_rows(src, dst, sem, rows, p, prio):
        copy(src, dst, sem, pl.multiple_of(p * rows, 8), rows, 0, src.shape[1], prio)

    c_x = pltpu.make_async_copy(x_hbm, x_v, wsem.at[4])
    c_wr = pltpu.make_async_copy(wr_hbm, wr_v, wsem.at[4])
    c_gw = pltpu.make_async_copy(gw_hbm, gw_v, wsem.at[4])

    strided(D // 8 * 3, 20, 0, 20, issue_wq)
    c_x.start(priority=0)
    c_wr.start(priority=1)
    c_gw.start(priority=0)
    strided(D // 8, 20, 0, 20, functools.partial(issue_rows, wg_hbm, wg_v, wsem.at[1], 8))
    strided(D // 8, 20, 0, 20, functools.partial(issue_rows, wu_hbm, wu_v, wsem.at[2], 8))
    start_units(0, 2)

    c_x.wait()
    c_wr.wait()
    c_gw.wait()
    wait_all(wq_v, wsem.at[0])
    x1 = x_v[0]
    x8 = jnp.broadcast_to(x1, (8, D))
    q = _rb(jnp.dot(x8, wq_v[...], preferred_element_type=F32))
    for h in range(H):
        q_v[h] = q[:, h * DH:(h + 1) * DH]

    wo_pieces = H * DH // 24
    issue_wo = functools.partial(issue_rows, wo_hbm, wo_v, wsem.at[3], 24)
    strided(wo_pieces, 16, 0, 4, issue_wo)

    wait_all(wg_v, wsem.at[1])
    wait_all(wu_v, wsem.at[2])
    xf = x1.astype(F32)
    wr = wr_v[...].reshape(1, D).astype(F32)
    gw = gw_v[...].reshape(1, D).astype(F32)
    r_sel = jax.nn.sigmoid(jnp.sum(xf * wr, axis=-1, keepdims=True))
    g = jax.nn.sigmoid(jnp.sum(xf * gw, axis=-1, keepdims=True))
    gate = jnp.dot(x8, wg_v[...], preferred_element_type=F32)
    up = jnp.dot(x8, wu_v[...], preferred_element_type=F32)
    hmid = _rb(jax.nn.silu(gate) * up)
    for j in range(N_DOWN):
        hm_v[j] = hmid[:, j * down_rows:(j + 1) * down_rows]

    strided(wo_pieces, 16, 4, 16, issue_wo)
    start_units(2, 2 * NBUF)
    wait_all(wo_v, wsem.at[3])

    scale = np.float32(DH ** -0.5)

    def start_down():
        rows = 24
        half = down_rows // rows // 2

        @pl.loop(0, N_DOWN)
        def _(j):
            for i in range(half):
                for t in range(2):
                    r = pl.multiple_of(j * down_rows + (t * half + i) * rows, 8)
                    copy(wd_hbm, wd_v, dsem.at[j], r, rows, 0, D, t)

    def head(h, acc):
        slot = h % NBUF
        wait_all(kbuf.at[slot], ksem.at[slot])
        qh = q_v[h].astype(BF16)
        s = jnp.dot(qh, kbuf[slot], preferred_element_type=F32) * scale

        @pl.when(h + NBUF < H)
        def _():
            start_kv(k_hbm, kbuf, ksem, h + NBUF, slot)

        m = jnp.max(s, axis=-1, keepdims=True)
        p = jnp.exp(s - m)
        l = jnp.sum(p, axis=-1, keepdims=True)
        wait_all(vbuf.at[slot], vsem.at[slot])
        pv = jax.lax.dot_general(p.astype(BF16), vbuf[slot], (((1,), (1,)), ((), ())),
                                 preferred_element_type=F32)

        @pl.when(h + NBUF < H)
        def _():
            start_kv(v_hbm, vbuf, vsem, h + NBUF, slot)

        @pl.when(h + NBUF == H)
        def _():
            start_down()

        o = (pv / l).astype(BF16)
        row0 = pl.multiple_of(h * DH, 64)
        return acc + jnp.dot(o, wo_v[pl.ds(row0, DH), :], preferred_element_type=F32)

    acc = jax.lax.fori_loop(0, H, head, jnp.zeros((8, D), F32))

    ga = g * acc[0:1]
    omg = 1.0 - g
    base = xf + xf * 0.0

    def down(j, y):
        rows = pl.ds(pl.multiple_of(j * down_rows, down_rows), down_rows)
        wait_all(wd_v.at[rows, :], dsem.at[j])
        return y + jnp.dot(hm_v[j].astype(BF16), wd_v[rows, :], preferred_element_type=F32)

    y = jax.lax.fori_loop(0, N_DOWN, down, jnp.zeros((8, D), F32))
    b = base + y[0:1] * r_sel
    o_ref[0] = (ga + omg * b).astype(o_ref.dtype)


@jax.jit
def pallas_gated_mix__sliding_block_cached__moe_arch_mod__decode_kernel(
    A_x: jax.Array,
    A_k_cache: jax.Array,
    A_v_cache: jax.Array,
    A_wq: jax.Array,
    A_wo: jax.Array,
    B_x: jax.Array,
    B_w_r: jax.Array,
    B_w_gate: jax.Array,
    B_w_up: jax.Array,
    B_w_down: jax.Array,
    gate_w: jax.Array,
):
    del B_x
    Bsz, Sq, D = A_x.shape
    Hkv, Sk = A_k_cache.shape[1], A_k_cache.shape[2]
    W = min(4096, max(256, Sk // 4))
    F = B_w_gate.shape[1]
    assert (Bsz, Sq) == (1, 1) and Hkv == HQ and A_k_cache.shape[3] == DH
    assert W % KV_LANES == 0 and (Sk - W) % 128 == 0

    any_spec = pl.BlockSpec(memory_space=pl.ANY)
    return pl.pallas_call(
        functools.partial(_kernel, s0=Sk - W, w=W),
        in_specs=[any_spec] * 10,
        out_specs=pl.BlockSpec(memory_space=pltpu.VMEM),
        out_shape=jax.ShapeDtypeStruct((Bsz, Sq, D), A_x.dtype),
        scratch_shapes=[
            pltpu.VMEM((1, 1, D), BF16),
            pltpu.VMEM((D,), BF16),
            pltpu.VMEM((D,), BF16),
            pltpu.VMEM((D, HQ * DH), BF16),
            pltpu.VMEM((HQ * DH, D), BF16),
            pltpu.VMEM((D, F), BF16),
            pltpu.VMEM((D, F), BF16),
            pltpu.VMEM((F, D), BF16),
            pltpu.VMEM((NBUF, DH, W), BF16),
            pltpu.VMEM((NBUF, DH, W), BF16),
            pltpu.VMEM((HQ, 8, DH), F32),
            pltpu.VMEM((N_DOWN, 8, F // N_DOWN), F32),
            pltpu.SemaphoreType.DMA((5,)),
            pltpu.SemaphoreType.DMA((N_DOWN,)),
            pltpu.SemaphoreType.DMA((NBUF,)),
            pltpu.SemaphoreType.DMA((NBUF,)),
        ],
        compiler_params=pltpu.CompilerParams(vmem_limit_bytes=64 * 1024 * 1024),
        name="gated_mix_decode",
    )(A_x, A_k_cache.transpose(0, 1, 3, 2), A_v_cache.transpose(0, 1, 3, 2), A_wq, A_wo,
      B_w_r, B_w_gate, B_w_up, B_w_down, gate_w)
```

```python
import functools

import jax
import jax.numpy as jnp
import numpy as np
import jax.experimental.pallas as pl
import jax.experimental.pallas.tpu as pltpu

HQ, DH = 32, 192
F32, BF16 = jnp.float32, jnp.bfloat16

NBUF = 2
KV_ROWS, KV_LANES = 32, 512
N_DOWN = 4


def _rb(v):
    return v.astype(BF16).astype(F32)


def _kernel(x_hbm, k_hbm, v_hbm, wq_hbm, wo_hbm, wr_hbm, wg_hbm, wu_hbm, wd_hbm, gw_hbm,
            o_ref,
            x_v, wr_v, gw_v, wq_v, wo_v, wg_v, wu_v, wd_v, kbuf, vbuf, q_v, hm_v,
            wsem, dsem, ksem, vsem, *, s0, w):
    H = HQ
    D = x_hbm.shape[-1]
    Fd = wg_hbm.shape[1]
    down_rows = Fd // N_DOWN

    def copy(src, dst, sem, r, nr, c, nc, prio):
        pltpu.make_async_copy(src.at[pl.ds(r, nr), pl.ds(c, nc)],
                              dst.at[pl.ds(r, nr), pl.ds(c, nc)], sem).start(priority=prio)

    def wait_all(dst, sem):
        pltpu.make_async_copy(dst, dst, sem).wait()

    def strided(n_pieces, stride, j0, j1, issue):
        inner = n_pieces // stride
        assert inner * stride == n_pieces and inner % 2 == 0

        @pl.loop(j0, j1)
        def _(j):
            for i in range(inner):
                issue(i * stride + j, i % 2)

    def start_kv(src, dst, sem, h, slot):
        for c in range(0, w, KV_LANES):
            for r0 in range(0, DH // 2, KV_ROWS):
                for prio in range(2):
                    r = r0 + prio * (DH // 2)
                    pltpu.make_async_copy(
                        src.at[0, h, pl.ds(r, KV_ROWS), pl.ds(s0 + c, KV_LANES)],
                        dst.at[slot, pl.ds(r, KV_ROWS), pl.ds(c, KV_LANES)],
                        sem.at[slot]).start(priority=prio)

    def start_units(lo, hi):
        @pl.loop(lo, hi)
        def _(u):
            h = u >> 1

            @pl.when((u & 1) == 0)
            def _():
                start_kv(k_hbm, kbuf, ksem, h, h)

            @pl.when((u & 1) == 1)
            def _():
                start_kv(v_hbm, vbuf, vsem, h, h)

    wq_cols = H * DH // 3

    def issue_wq(p, prio):
        rt = (p * 43691) >> 17
        c = p - 3 * rt
        copy(wq_hbm, wq_v, wsem.at[0], pl.multiple_of(rt * 8, 8), 8,
             pl.multiple_of(c * wq_cols, 128), wq_cols, prio)

    def issue_rows(src, dst, sem, rows, p, prio):
        copy(src, dst, sem, pl.multiple_of(p * rows, 8), rows, 0, src.shape[1], prio)

    c_x = pltpu.make_async_copy(x_hbm, x_v, wsem.at[4])
    c_wr = pltpu.make_async_copy(wr_hbm, wr_v, wsem.at[4])
    c_gw = pltpu.make_async_copy(gw_hbm, gw_v, wsem.at[4])

    strided(D // 8 * 3, 20, 0, 20, issue_wq)
    c_x.start(priority=0)
    c_wr.start(priority=1)
    c_gw.start(priority=0)
    strided(D // 8, 10, 0, 10, functools.partial(issue_rows, wg_hbm, wg_v, wsem.at[1], 8))
    strided(D // 8, 10, 0, 10, functools.partial(issue_rows, wu_hbm, wu_v, wsem.at[2], 8))
    start_units(0, 2)

    c_x.wait()
    c_wr.wait()
    c_gw.wait()
    wait_all(wq_v, wsem.at[0])
    x1 = x_v[0]
    x8 = jnp.broadcast_to(x1, (8, D))
    q = _rb(jnp.dot(x8, wq_v[...], preferred_element_type=F32))
    for h in range(H):
        q_v[h] = q[:, h * DH:(h + 1) * DH]

    wo_pieces = H * DH // 24
    issue_wo = functools.partial(issue_rows, wo_hbm, wo_v, wsem.at[3], 24)
    strided(wo_pieces, 16, 0, 4, issue_wo)

    wait_all(wg_v, wsem.at[1])
    wait_all(wu_v, wsem.at[2])
    xf = x1.astype(F32)
    wr = wr_v[...].reshape(1, D).astype(F32)
    gw = gw_v[...].reshape(1, D).astype(F32)
    r_sel = jax.nn.sigmoid(jnp.sum(xf * wr, axis=-1, keepdims=True))
    g = jax.nn.sigmoid(jnp.sum(xf * gw, axis=-1, keepdims=True))
    gate = jnp.dot(x8, wg_v[...], preferred_element_type=F32)
    up = jnp.dot(x8, wu_v[...], preferred_element_type=F32)
    hmid = _rb(jax.nn.silu(gate) * up)
    for j in range(N_DOWN):
        hm_v[j] = hmid[:, j * down_rows:(j + 1) * down_rows]

    strided(wo_pieces, 16, 4, 16, issue_wo)
    start_units(2, 2 * NBUF)
    wait_all(wo_v, wsem.at[3])

    scale = np.float32(DH ** -0.5)

    def start_down():
        rows = 24
        half = down_rows // rows // 2

        @pl.loop(0, N_DOWN)
        def _(j):
            for i in range(half):
                for t in range(2):
                    r = pl.multiple_of(j * down_rows + (t * half + i) * rows, 8)
                    copy(wd_hbm, wd_v, dsem.at[j], r, rows, 0, D, t)

    def head(h, acc):
        slot = h % NBUF
        wait_all(kbuf.at[slot], ksem.at[slot])
        qh = q_v[h].astype(BF16)
        s = jnp.dot(qh, kbuf[slot], preferred_element_type=F32) * scale

        @pl.when(h + NBUF < H)
        def _():
            start_kv(k_hbm, kbuf, ksem, h + NBUF, slot)

        m = jnp.max(s, axis=-1, keepdims=True)
        p = jnp.exp(s - m)
        l = jnp.sum(p, axis=-1, keepdims=True)
        wait_all(vbuf.at[slot], vsem.at[slot])
        pv = jax.lax.dot_general(p.astype(BF16), vbuf[slot], (((1,), (1,)), ((), ())),
                                 preferred_element_type=F32)

        @pl.when(h + NBUF < H)
        def _():
            start_kv(v_hbm, vbuf, vsem, h + NBUF, slot)

        @pl.when(h + NBUF == H)
        def _():
            start_down()

        o = (pv / l).astype(BF16)
        row0 = pl.multiple_of(h * DH, 64)
        return acc + jnp.dot(o, wo_v[pl.ds(row0, DH), :], preferred_element_type=F32)

    acc = jax.lax.fori_loop(0, H, head, jnp.zeros((8, D), F32))

    ga = g * acc[0:1]
    omg = 1.0 - g
    base = xf + xf * 0.0

    def down(j, y):
        rows = pl.ds(pl.multiple_of(j * down_rows, down_rows), down_rows)
        wait_all(wd_v.at[rows, :], dsem.at[j])
        return y + jnp.dot(hm_v[j].astype(BF16), wd_v[rows, :], preferred_element_type=F32)

    y = jax.lax.fori_loop(0, N_DOWN, down, jnp.zeros((8, D), F32))
    b = base + y[0:1] * r_sel
    o_ref[0] = (ga + omg * b).astype(o_ref.dtype)


@jax.jit
def pallas_gated_mix__sliding_block_cached__moe_arch_mod__decode_kernel(
    A_x: jax.Array,
    A_k_cache: jax.Array,
    A_v_cache: jax.Array,
    A_wq: jax.Array,
    A_wo: jax.Array,
    B_x: jax.Array,
    B_w_r: jax.Array,
    B_w_gate: jax.Array,
    B_w_up: jax.Array,
    B_w_down: jax.Array,
    gate_w: jax.Array,
):
    del B_x
    Bsz, Sq, D = A_x.shape
    Hkv, Sk = A_k_cache.shape[1], A_k_cache.shape[2]
    W = min(4096, max(256, Sk // 4))
    F = B_w_gate.shape[1]
    assert (Bsz, Sq) == (1, 1) and Hkv == HQ and A_k_cache.shape[3] == DH
    assert W % KV_LANES == 0 and (Sk - W) % 128 == 0

    any_spec = pl.BlockSpec(memory_space=pl.ANY)
    return pl.pallas_call(
        functools.partial(_kernel, s0=Sk - W, w=W),
        in_specs=[any_spec] * 10,
        out_specs=pl.BlockSpec(memory_space=pltpu.VMEM),
        out_shape=jax.ShapeDtypeStruct((Bsz, Sq, D), A_x.dtype),
        scratch_shapes=[
            pltpu.VMEM((1, 1, D), BF16),
            pltpu.VMEM((D,), BF16),
            pltpu.VMEM((D,), BF16),
            pltpu.VMEM((D, HQ * DH), BF16),
            pltpu.VMEM((HQ * DH, D), BF16),
            pltpu.VMEM((D, F), BF16),
            pltpu.VMEM((D, F), BF16),
            pltpu.VMEM((F, D), BF16),
            pltpu.VMEM((NBUF, DH, W), BF16),
            pltpu.VMEM((NBUF, DH, W), BF16),
            pltpu.VMEM((HQ, 8, DH), F32),
            pltpu.VMEM((N_DOWN, 8, F // N_DOWN), F32),
            pltpu.SemaphoreType.DMA((5,)),
            pltpu.SemaphoreType.DMA((N_DOWN,)),
            pltpu.SemaphoreType.DMA((NBUF,)),
            pltpu.SemaphoreType.DMA((NBUF,)),
        ],
        compiler_params=pltpu.CompilerParams(vmem_limit_bytes=64 * 1024 * 1024),
        name="gated_mix_decode",
    )(A_x, A_k_cache.transpose(0, 1, 3, 2), A_v_cache.transpose(0, 1, 3, 2), A_wq, A_wo,
      B_w_r, B_w_gate, B_w_up, B_w_down, gate_w)
```
